```python
import os as _os
_os.environ.setdefault("JAX_PLATFORMS", "cpu")
import jax
import jax.numpy as jnp

def _softmax(x, axis=-1):
    return jax.nn.softmax(x, axis=axis)
def _gelu(x):
    return jax.nn.gelu(x, approximate=True)
def _silu(x):
    return jax.nn.silu(x)
def _sigmoid(x):
    return jax.nn.sigmoid(x)
def _layernorm(x, axis=-1, eps=1e-5):
    m = jnp.mean(x, axis=axis, keepdims=True)
    v = jnp.var(x, axis=axis, keepdims=True)
    return (x - m) / jnp.sqrt(v + eps)
def _scatter_add(tgt, idx, src, axis=0):
    return tgt.at[idx].add(src)
def _segment_sum(src, seg, n):
    return jax.ops.segment_sum(src, seg, n)
class _Rng:
    def __init__(self, key):
        self._k = key
    def _next(self):
        self._k, sub = jax.random.split(self._k)
        return sub
    def normal(self, shape):
        return jax.random.normal(self._next(), shape, dtype=jnp.bfloat16)
    def randint(self, lo, hi, shape):
        return jax.random.randint(self._next(), shape, lo, hi, dtype=jnp.int32)
    def uniform(self, shape, lo=0.0, hi=1.0):
        return jax.random.uniform(self._next(), shape, jnp.bfloat16, lo, hi)
    def permutation(self, n):
        return jax.random.permutation(self._next(), n)


kernel_name = 'standalone__mha_block_cached__near_ridge'

def setup_inputs():
    _rng = _Rng(jax.random.key(int.from_bytes(__import__("os").urandom(4), "little")))
    _w = (lambda a: (lambda t: t.astype(jnp.bfloat16) if jnp.issubdtype(t.dtype, jnp.floating) else t)(jnp.asarray(a)))
    B, Sq, D = 8, 144, 448
    H, Sk, Dh = 16, 2048, 256
    return {
        "x": _w((lambda *s: _rng.normal(s) * 0.8)(B, Sq, D)),
        "k_cache": _w((lambda *s: _rng.normal(s) * 0.8)(B, H, Sk, Dh)),
        "v_cache": _w((lambda *s: _rng.normal(s) * 0.05)(B, H, Sk, Dh)),
        "wq": _w((lambda *s: _rng.normal(s) * 0.8)(D, H * Dh) * (D ** -0.5)),
        "wo": _w((lambda *s: _rng.normal(s) * 0.05)(H * Dh, D) * ((H * Dh) ** -0.5)),
    }

def reference(x, k_cache, v_cache, wq, wo):
    B, Sq, D = x.shape
    H, Dh = 16, 256
    q = (lambda x, *d: x.transpose(*d))((x @ wq).reshape(B, Sq, H, Dh), 0, 2, 1, 3)
    scores = jnp.einsum("bhqd,bhkd->bhqk", q, k_cache) * (Dh ** -0.5)
    p = _softmax(scores, axis=-1)
    o = jnp.einsum("bhqk,bhkd->bhqd", p, v_cache)
    return (lambda x, *d: x.transpose(*d))(o, 0, 2, 1, 3).reshape(B, Sq, H * Dh) @ wo
```

```python
import functools
import jax, jax.numpy as jnp
from jax import lax
from jax.experimental import pallas as pl
from jax.experimental.pallas import tpu as pltpu

NT = (((1,), (1,)), ((), ()))
LOG2E = 1.4426950408889634
B, Sq, D, H, Sk, Dh = 8, 144, 448, 16, 2048, 256
N = B * H

def lane_fold(x, op):
    r = x[:, 0:128]
    for c in range(128, x.shape[1], 128):
        r = op(r, x[:, c:c + 128])
    return r

def make_sched(W, jD, jS):
    PW = 4 // W; PRE = W - 1; M_W = 2 * jD; M_S = 2 * jS
    NM = M_S + 4 * (N - jS)
    def tri(lst):
        blocks = []
        for h, c0, n in lst:
            blocks += [(h, c0 + 4 * i) for i in range(n // 4)]
        out = []
        for m in range(len(blocks) // 4):
            g = blocks[4 * m:4 * m + 4]
            ent = []
            for p, (h, c) in enumerate(g):
                same = [x for x in g if x[0] == h]
                ent.append((h, same[0][1] + same.index((h, c)), len(same)))
            out.append(ent)
        return out
    up = tri([(h, 32 - 8 * (W - 1 - h) * PW, 8 * (W - 1 - h) * PW) for h in range(W - 1)])
    c_dn = ((M_W - 2 * PRE) * 4 * PW) & 31
    dn_l = []
    for h in range(W - 1):
        n = 8 * (h + 1) * PW
        n1 = min(n, 32 - c_dn)
        dn_l.append((jD - W + 1 + h, c_dn, n1))
        if n > n1: dn_l.append((jD - W + 1 + h, 0, n - n1))
    dn = tri(dn_l)
    def sched(m, where):
        out = []
        for pos in range(4):
            w, sub = pos // PW, pos % PW
            t = m + PRE - 2 * w
            j = (t >> W.bit_length()) * W + w
            c = ((m - PRE) & (2 * W - 1)) * (4 * PW) + sub
            st = PW
            for k_, ent in enumerate(up):
                sel = m == k_
                j = where(sel, ent[pos][0], j); c = where(sel, ent[pos][1], c); st = where(sel, ent[pos][2], st)
            for k_, ent in enumerate(dn):
                sel = m == M_W - PRE + k_
                j = where(sel, ent[pos][0], j); c = where(sel, ent[pos][1], c); st = where(sel, ent[pos][2], st)
            if W > 1:
                sel = m >= M_W
                j = where(sel, m >> 1, j); c = where(sel, (m & 1) * 16 + pos, c); st = where(sel, 4, st)
            if jS < N:
                j = where(m >= M_S, jS + ((m - M_S) >> 2), j)
            out.append((j, c, st))
        vk = (m < NM) & ((m < M_S) | (((m - M_S) & 2) == 0))
        vv = (m < NM) & ((m < M_S) | (((m - M_S) & 2) != 0))
        return out, vk, vv
    return sched, NM

def slots_in_step(i, skips):
    return 1 if i in skips else 2

def check_schedule(W, ns, pm, skips, jD, jS):
    sched, NM = make_sched(W, jD, jS)
    seen = {}
    def issue(m, step):
        lst, vk, vv = sched(m, lambda s_, a, b: a if s_ else b)
        for (j, c) in [(j, c + t * st) for (j, c, st) in lst for t in range(4)]:
            for w, ok in ((0, vk), (1, vv)):
                if not ok: continue
                assert (w, j, c) not in seen, ("dup", w, j, c, m)
                assert 0 <= j < N and 0 <= c < 32, (j, c, m)
                assert j - ns < step, ("slot busy", j, step)
                seen[(w, j, c)] = step
    for m in range(pm): issue(m, -1)
    m0 = pm
    for i in range(N):
        for w in (0, 1):
            for c in range(32):
                assert (w, i, c) in seen, ("deadlock", w, i, c)
        n = slots_in_step(i, skips)
        for t in range(n): issue(m0 + t, i)
        m0 += n
    assert len(seen) == 2 * N * 32
    return max(seen.values())

def make(W=2, ns=8, pm=6, skips=(), jD=124, jS=126, issue=("end", "end"), kc=256, vc=256, order="K qk V q pv o", nodma=False, flags=None,
         defer=True, wstep=None):
    assert ns & (ns - 1) == 0
    order = order.split()
    sched, NM = make_sched(W, jD, jS)
    last = check_schedule(W, ns, pm, skips, jD, jS)
    if wstep is None: wstep = min(last, N - 2)

    def kern(x_hbm, k_hbm, v_hbm, wq_hbm, wo_hbm, o_hbm, kbuf, vbuf, xbuf, wq, wo, acc, obuf, qs, os_, sem, wsem, osem):
        def munit(m):
            lst, vk, vv = sched(m, jnp.where)
            refs = []
            for (j, c, stp) in lst:
                refs.append((j, j & (ns - 1), c * 32, stp * 32))
            for t in range(4):
                for (j, slot, r0, stp) in refs:
                    r = pl.ds(pl.multiple_of(r0 + stp * t, 32), 32)
                    @pl.when(vk)
                    def _():
                        pltpu.make_async_copy(k_hbm.at[j, :, r, :], kbuf.at[slot, :, r, :], sem.at[slot, 0]).start(priority=0)
                    @pl.when(vv)
                    def _():
                        pltpu.make_async_copy(v_hbm.at[j, :, r, :], vbuf.at[slot, :, r, :], sem.at[slot, 1]).start(priority=1)

        @pl.loop(0, 28)
        def _(r):
            r0 = pl.multiple_of(r * 8, 8)
            for c in range(0, 4096, 1024):
                pltpu.make_async_copy(wq_hbm.at[:, pl.ds(r0, 8), pl.ds(c, 1024)], wq.at[:, pl.ds(r0, 8), pl.ds(c, 1024)], wsem.at[0]).start(priority=0)
                pltpu.make_async_copy(wo_hbm.at[:, pl.ds(r0, 8), pl.ds(c, 1024)], wo.at[:, pl.ds(r0, 8), pl.ds(c, 1024)], wsem.at[1]).start(priority=1)
        @pl.loop(0, 9)
        def _(r):
            r0 = pl.multiple_of(r * 16, 16)
            for b in range(0, B, 2):
                pltpu.make_async_copy(x_hbm.at[pl.ds(b, 2), pl.ds(r0, 16)], xbuf.at[pl.ds(b, 2), pl.ds(r0, 16)], wsem.at[2]).start(priority=(b >> 1) & 1)
        if not nodma:
            @pl.loop(0, pm)
            def _(m):
                munit(m)
        acc[...] = jnp.zeros(acc.shape, acc.dtype)
        os_[...] = jnp.zeros(os_.shape, os_.dtype)
        pltpu.make_async_copy(wq, wq, wsem.at[0]).wait()
        pltpu.make_async_copy(wo, wo, wsem.at[1]).wait()
        pltpu.make_async_copy(xbuf, xbuf, wsem.at[2]).wait()

        def qproj(j):
            off = pl.multiple_of((j & 15) * 256, 256)
            w = wq[:, :, pl.ds(off, 256)].reshape(D, 256)
            q = jnp.dot(xbuf[j >> 4], w, preferred_element_type=jnp.float32)
            return (q * (LOG2E / 16.0)).astype(jnp.bfloat16)
        def oproj(o, j):
            off = pl.multiple_of((j & 15) * 256, 256)
            w = wo[:, :, pl.ds(off, 256)].reshape(D, 256)
            return lax.dot_general(o, w, NT, preferred_element_type=jnp.float32)
        def accum(y, j):
            a = jnp.where((j & 15) == 0, 0.0, acc[...]) + y
            acc[...] = a
            obuf[j >> 4] = a.astype(obuf.dtype)

        qs[...] = qproj(0)
        skew_o = "op" in order

        def body(i, m0):
            slot = i & (ns - 1)
            skip = None
            for s_ in skips:
                skip = (i == s_) if skip is None else (skip | (i == s_))
            def at(name):
                for t, nm in enumerate(issue):
                    if nm == name:
                        if t == 1 and skip is not None:
                            munit(jnp.where(skip, NM, m0 + t))
                        else:
                            munit(m0 + t)
            st = {}
            q = qs[...]
            for tok in order:
                if tok == "K":
                    if not nodma: pltpu.make_async_copy(kbuf.at[slot], kbuf.at[slot], sem.at[slot, 0]).wait()
                elif tok == "V":
                    if not nodma: pltpu.make_async_copy(vbuf.at[slot], vbuf.at[slot], sem.at[slot, 1]).wait()
                elif tok == "qk":
                    ss = []
                    mx = None
                    for t in range(Sk // kc):
                        hf, r0 = divmod(t * kc, Sk // 2)
                        s = lax.dot_general(q, kbuf[slot, hf, pl.ds(r0, kc), :], NT, preferred_element_type=jnp.float32)
                        ss.append(s)
                        mt = lane_fold(s, jnp.maximum)
                        mx = mt if mx is None else jnp.maximum(mx, mt)
                        at(f"qk{t}")
                    st["s"] = jnp.concatenate(ss, axis=1)
                    st["mx"] = mx
                elif tok == "q":
                    qs[...] = qproj(jnp.minimum(i + 1, N - 1))
                elif tok == "op":
                    jp = jnp.maximum(i - 1, 0)
                    accum(oproj(os_[...], jp), jp)
                elif tok == "pv":
                    o = l = None
                    st["m"] = jnp.max(st["mx"], axis=-1, keepdims=True)
                    for t in range(Sk // vc):
                        hf, r0 = divmod(t * vc, Sk // 2)
                        p = jnp.exp2(st["s"][:, t * vc:(t + 1) * vc] - st["m"])
                        lt = lane_fold(p, jnp.add)
                        l = lt if l is None else l + lt
                        ot = jnp.dot(p.astype(jnp.bfloat16), vbuf[slot, hf, pl.ds(r0, vc), :], preferred_element_type=jnp.float32)
                        o = ot if o is None else o + ot
                        at(f"pv{t}")
                    l = jnp.sum(l, axis=-1, keepdims=True)
                    st["o"] = (o * (1.0 / l)).astype(jnp.bfloat16)
                    if skew_o:
                        os_[...] = st["o"]
                elif tok == "o":
                    accum(oproj(st["o"], i), i)
                else:
                    raise ValueError(tok)
                at(tok + "_")
            at("end")
            if defer:
                @pl.when(i == wstep)
                def _():
                    for b in range(B - 1):
                        pltpu.make_async_copy(obuf.at[b], o_hbm.at[b], osem.at[0]).start(priority=b & 1)
            return m0 + (2 if skip is None else jnp.where(skip, 1, 2))
        lax.fori_loop(0, N, body, jnp.int32(NM if nodma else pm))
        if skew_o:
            accum(oproj(os_[...], N - 1), N - 1)
        if defer:
            pltpu.make_async_copy(obuf.at[B - 1], o_hbm.at[B - 1], osem.at[0]).start()
        else:
            pltpu.make_async_copy(obuf, o_hbm, osem.at[0]).start()
        pltpu.make_async_copy(obuf, o_hbm, osem.at[0]).wait()

    def f(x, k, v, wq, wo):
        anyspec = pl.BlockSpec(memory_space=pl.ANY)
        return pl.pallas_call(
            kern,
            in_specs=[anyspec] * 5,
            out_specs=anyspec,
            out_shape=jax.ShapeDtypeStruct((B, Sq, D), x.dtype),
            scratch_shapes=[pltpu.VMEM((ns, 2, Sk // 2, Dh), jnp.bfloat16), pltpu.VMEM((ns, 2, Sk // 2, Dh), jnp.bfloat16),
                            pltpu.VMEM((B, Sq, D), jnp.bfloat16), pltpu.VMEM((2, D // 2, H * Dh), jnp.bfloat16), pltpu.VMEM((2, D // 2, H * Dh), jnp.bfloat16),
                            pltpu.VMEM((Sq, D), jnp.float32), pltpu.VMEM((B, Sq, D), jnp.bfloat16),
                            pltpu.VMEM((Sq, Dh), jnp.bfloat16), pltpu.VMEM((Sq, Dh), jnp.bfloat16),
                            pltpu.SemaphoreType.DMA((ns, 2)), pltpu.SemaphoreType.DMA((3,)), pltpu.SemaphoreType.DMA((1,))],
            compiler_params=pltpu.CompilerParams(vmem_limit_bytes=110 * 1024 * 1024, disable_bounds_checks=True, flags=flags),
        )(x, k.reshape(N, 2, Sk // 2, Dh), v.reshape(N, 2, Sk // 2, Dh), wq.reshape(2, D // 2, H * Dh), wo.T.reshape(2, D // 2, H * Dh))
    return f


_impl = make(W=4, order="K qk V q pv o", issue=("qk3", "pv3"), pm=7, skips=(113, 117, 121), jD=116, jS=127)


@jax.jit
def pallas_standalone__mha_block_cached__near_ridge_kernel(x, k_cache, v_cache, wq, wo):
    return _impl(x, k_cache, v_cache, wq, wo)
```

```python
import jax
import jax.numpy as jnp
from jax import lax
from jax.experimental import pallas as pl
from jax.experimental.pallas import tpu as pltpu

B, SQ, D = 8, 144, 448
H, SK, DH = 16, 2048, 256
N = B * H
HALF = SK // 2
PIECE = 32
BLOCK = 4 * PIECE
SLOTS = 8
KEYS = 256
W_GROUPS = 7
Q_SCALE = DH**-0.5 * 1.4426950408889634
NT = (((1,), (1,)), ((), ()))

J_PAIR = 114
J_HALF = 124
J_TAIL = 120
LEAD = 12
SKEW = 26
QUIET = (121, 123, 125)
LAST_SPLIT = 640

SEM_W, SEM_LAST, SEM_OUT, NUM_SEMS = 4 * SLOTS, 4 * SLOTS + 3, 4 * SLOTS + 4, 4 * SLOTS + 5


def _window_positions(m, first, width, blocks):
    lanes, stagger = 4 // width, blocks // 4
    period = stagger * width
    positions = []
    for pos in range(4):
        w, sub = divmod(pos, lanes)
        turn = (m + stagger * (width - 1 - w)) >> (period.bit_length() - 1)
        positions.append((first + turn * width + w, (m & (period - 1)) * (BLOCK * lanes) + PIECE * sub, PIECE * lanes))
    return positions


def _run(obj, first_block, units):
    assert first_block % 4 == 0
    return [[(obj, BLOCK * ((first_block + 4 * u) % 16) + PIECE * pos, BLOCK) for pos in range(4)] for u in range(units)]


def _copies(kind, positions):
    return [(kind, kv, obj, row + step * t, kv) for t in range(4) for obj, row, step in positions for kv in (0, 1)]


def _make_plan():
    slabs = J_PAIR // 2
    left = 4 * (slabs - 3) % 16
    pair = _run(0, 4, 3) + _run(1, 8, 2) + _run(2, 12, 1)
    pair += [_window_positions(m, 0, 4, 16) for m in range(4 * (slabs - 3))]
    pair += _run(slabs - 3, left, 1) + _run(slabs - 2, left, 2) + _run(slabs - 1, left, 3)

    heads = J_HALF - J_PAIR
    half = _run(J_PAIR, 4, 1)
    half += [_window_positions(m, J_PAIR, 2, 8) for m in range(2 * (heads - 1))]
    half += _run(J_HALF - 1, 4 * (heads - 1) % 8, 1)

    rest = [("half", kv, j, row) for j in range(J_HALF, N) for kv in (0, 1) for row in range(0, HALF, PIECE)]
    queues = ([], [])
    for k, copy in enumerate(rest):
        if k >= len(rest) - 2 * SKEW:
            queue = int(k >= len(rest) - SKEW)
        else:
            queue = 0 if k < SKEW else (k - SKEW + 1) % 2
        queues[queue].append(copy + (queue,))
    rest = [q[k] for k in range(len(queues[0])) for q in queues if k < len(q)]

    units = [_copies("pair", p) for p in pair] + [_copies("half", p) for p in half]
    return pair, half, units + [rest[k : k + 32] for k in range(0, len(rest), 32)]


PAIR_UNITS, HALF_UNITS, UNITS = _make_plan()
J_SWITCH = (len(PAIR_UNITS) - LEAD) // 2


def _half_units_before(j):
    return (3 * (j - J_SWITCH)) >> 1


def _check_plan():
    unit_of = {}
    for n, unit in enumerate(UNITS):
        for kind, kv, obj, row, _ in unit:
            for i in (0, 1):
                key = (kv, 2 * obj + i, row) if kind == "pair" else (kv, obj, i * HALF + row)
                assert key not in unit_of
                unit_of[key] = n
    assert set(unit_of) == {(kv, j, row) for kv in (0, 1) for j in range(N) for row in range(0, SK, PIECE)}
    assert LEAD + 2 * J_SWITCH == len(PAIR_UNITS) and _half_units_before(J_TAIL) < len(HALF_UNITS)
    assert 2 + 3 * (J_SWITCH // 2) >= N and J_SWITCH <= J_PAIR <= J_TAIL <= J_HALF
    started = LEAD
    for j in range(N):
        awaited = (j,) if j >= J_PAIR else (j & ~1, j | 1)
        assert all(unit_of[kv, i, row] < started for kv in (0, 1) for i in awaited for row in range(0, SK, PIECE))
        if j < J_SWITCH:
            count = 2
        elif j < J_TAIL:
            count = _half_units_before(j + 1) - _half_units_before(j)
        else:
            count = 0 if j == N - 1 else 1 if j in QUIET else 2
        for unit in UNITS[started : started + count]:
            assert all((obj if kind == "pair" else obj // 2) - SLOTS < j // 2 for kind, _, obj, _, _ in unit)
        started += count
    assert started >= len(UNITS)


_check_plan()


def _lane_fold(x, op):
    out = x[:, :128]
    for c in range(128, x.shape[1], 128):
        out = op(out, x[:, c : c + 128])
    return out


def _kernel(
    x_hbm, k_hbm, v_hbm, wq_hbm, wo_hbm, out_hbm,
    k_buf, v_buf, x_buf, wq_buf, wo_buf, q_buf, o_buf, acc, out_buf, sems,
):
    kv_hbm, kv_buf = (k_hbm, v_hbm), (k_buf, v_buf)

    def kv_sem(slot, e, kv):
        return sems.at[4 * slot + 2 * e + kv]

    def start_copy(kind, kv, obj, row, queue):
        if kind == "pair":
            slab, sem = obj, kv_sem(obj % SLOTS, 0, kv)
            ix = (slice(None), row // HALF, pl.ds(row % HALF, PIECE))
        else:
            slab, sem = obj // 2, kv_sem(obj // 2 % SLOTS, obj % 2, kv)
            ix = (obj % 2, slice(None), pl.ds(row, PIECE))
            if (kv, obj) == (1, N - 1) and row >= LAST_SPLIT:
                sem = sems.at[SEM_LAST]
        src, dst = kv_hbm[kv].at[(slab,) + ix], kv_buf[kv].at[(slab % SLOTS,) + ix]
        pltpu.make_async_copy(src, dst, sem).start(priority=queue)

    def start_unit(kind, m, positions, special, enabled=None):
        for k, other in special:
            positions = [tuple(jnp.where(m == k, a, b) for a, b in zip(p, q)) for p, q in zip(other, positions)]
        if kind == "pair":
            bases = [(obj, row >> 10, row & (HALF - 1), step) for obj, row, step in positions]
        else:
            bases = [(obj >> 1, obj & 1, row, step) for obj, row, step in positions]
        for t in range(4):
            for slab, mid, row, step in bases:
                rows, slot = pl.ds(pl.multiple_of(row + step * t, PIECE), PIECE), slab & (SLOTS - 1)
                ix = (slice(None), mid, rows) if kind == "pair" else (mid, slice(None), rows)

                def start():
                    for kv in (0, 1):
                        src, dst = kv_hbm[kv].at[(slab,) + ix], kv_buf[kv].at[(slot,) + ix]
                        sem = kv_sem(slot, 0 if kind == "pair" else mid, kv)
                        pltpu.make_async_copy(src, dst, sem).start(priority=kv)

                if enabled is None:
                    start()
                else:
                    pl.when(enabled)(start)

    def wait_filled(ref, sem):
        pltpu.make_async_copy(ref, ref, sem).wait()

    def head_cols(j):
        start = (j & (H - 1)) * DH
        return pl.ds(start if isinstance(start, int) else pl.multiple_of(start, DH), DH)

    def project_q(j):
        w = wq_buf[:, :, head_cols(j)].reshape(D, DH)
        q = jnp.dot(x_buf[j >> 4], w, preferred_element_type=jnp.float32)
        q_buf[j] = (q * Q_SCALE).astype(q_buf.dtype)

    def project_out(o, j):
        w = wo_buf[:, :, head_cols(j)].reshape(D, DH)
        y = lax.dot_general(o, w, NT, preferred_element_type=jnp.float32)
        if isinstance(j, int):
            y = y if j % H == 0 else acc[...] + y
            if j % H == H - 1:
                out_buf[j // H] = y.astype(out_buf.dtype)
            else:
                acc[...] = y
        else:
            y = jnp.where((j & (H - 1)) == 0, 0.0, acc[...]) + y
            acc[...] = y
            out_buf[j >> 4] = y.astype(out_buf.dtype)

    def key_chunks(lo, hi):
        return [(hf, r, min(KEYS, hi - r)) for hf in (0, 1) for r in range(lo, hi, KEYS)]

    def scores(st, j, midway):
        q = q_buf[j]
        for t, (hf, r, n) in enumerate(key_chunks(0, HALF)):
            k = k_buf[(j >> 1) & (SLOTS - 1), j & 1, hf, pl.ds(r, n), :]
            s = lax.dot_general(q, k, NT, preferred_element_type=jnp.float32)
            for c in range(0, n, 128):
                st[hf, r + c] = s[:, c : c + 128]
            top = _lane_fold(s, jnp.maximum)
            st["top"] = jnp.maximum(st["top"], top) if "top" in st else top
            if t == 3:
                midway()

    def row_max(st):
        if "max" not in st:
            st["max"] = jnp.max(st["top"], axis=-1, keepdims=True)
        return st["max"]

    def attend(st, j, lo, hi, midway):
        for t, (hf, r, n) in enumerate(key_chunks(lo, hi)):
            s = jnp.concatenate([st[hf, r + c] for c in range(0, n, 128)], axis=1)
            p = jnp.exp2(s - row_max(st))
            total = _lane_fold(p, jnp.add)
            st["sum"] = st["sum"] + total if "sum" in st else total
            v = v_buf[(j >> 1) & (SLOTS - 1), j & 1, hf, pl.ds(r, n), :]
            o = jnp.dot(p.astype(v.dtype), v, preferred_element_type=jnp.float32)
            st["o"] = st["o"] + o if "o" in st else o
            if t == 3:
                midway()

    def normalized(st):
        return (st["o"] * (1.0 / jnp.sum(st["sum"], axis=-1, keepdims=True))).astype(o_buf.dtype)

    def head(j, start_first, start_second):
        st = {}
        scores(st, j, start_first)
        project_out(o_buf[...], jnp.maximum(j - 1, 0))
        attend(st, j, 0, HALF, start_second)
        o_buf[...] = normalized(st)

    for r in range(0, D // W_GROUPS, 8):
        for c in range(0, H * DH, 1024):
            parts = [(pl.ds(g, 2), pl.ds(r, 8), pl.ds(c, 1024)) for g in range(0, W_GROUPS - 1, 2)]
            if c % 2048 == 0:
                parts.append((W_GROUPS - 1, pl.ds(r, 8), pl.ds(c, 2048)))
            for ix in parts:
                pltpu.make_async_copy(wq_hbm.at[ix], wq_buf.at[ix], sems.at[SEM_W]).start(priority=0)
                pltpu.make_async_copy(wo_hbm.at[ix], wo_buf.at[ix], sems.at[SEM_W + 1]).start(priority=1)
    x_parts = [(pl.ds(b, 2), pl.ds(r, 16)) for r in range(0, SQ, 16) for b in (0, 4, 2, 6)]
    for k, copy in enumerate(copy for unit in UNITS[:LEAD] for copy in unit):
        start_copy(*copy)
        if k % 8 == 7 and x_parts:
            for queue in (0, 1):
                ix = x_parts.pop(0)
                pltpu.make_async_copy(x_hbm.at[ix], x_buf.at[ix], sems.at[SEM_W + 2]).start(priority=queue)
    assert not x_parts
    acc[...] = jnp.zeros(acc.shape, acc.dtype)
    o_buf[...] = jnp.zeros(o_buf.shape, o_buf.dtype)
    for n, ref in enumerate((wq_buf, wo_buf, x_buf)):
        wait_filled(ref, sems.at[SEM_W + n])
    project_q(0)
    project_q(1)

    @pl.loop(0, J_SWITCH)
    def _(j):
        even, slot = (j & 1) == 0, (j >> 1) & (SLOTS - 1)
        ahead = 2 + 3 * (j >> 1)

        @pl.when(even & (ahead < N))
        def _():
            for t in range(3):
                project_q(ahead + t)

        @pl.when(even)
        def _():
            for kv in (0, 1):
                wait_filled(kv_buf[kv].at[slot], kv_sem(slot, 0, kv))

        def unit(m):
            drain = [(k, PAIR_UNITS[k]) for k in range(len(PAIR_UNITS) - 6, len(PAIR_UNITS))]
            start_unit("pair", m, _window_positions(m - 6, 0, 4, 16), drain)

        head(j, lambda: unit(LEAD + 2 * j), lambda: unit(LEAD + 2 * j + 1))

    @pl.loop(J_SWITCH, J_TAIL)
    def _(j):
        slot, e = (j >> 1) & (SLOTS - 1), j & 1

        @pl.when((j < J_PAIR) & (e == 0))
        def _():
            for kv in (0, 1):
                wait_filled(kv_buf[kv].at[slot], kv_sem(slot, 0, kv))

        @pl.when(j >= J_PAIR)
        def _():
            for kv in (0, 1):
                wait_filled(kv_buf[kv].at[slot, e], kv_sem(slot, e, kv))

        def unit(m, enabled=None):
            start_unit("half", m, _window_positions(m - 1, J_PAIR, 2, 8), [(0, HALF_UNITS[0])], enabled)

        m = _half_units_before(j)
        head(j, lambda: unit(m), lambda: unit(m + 1, _half_units_before(j + 1) == m + 2))

    pending = UNITS[len(PAIR_UNITS) + _half_units_before(J_TAIL) :]

    def start_next():
        for copy in pending.pop(0) if pending else ():
            start_copy(*copy)

    def nothing():
        pass

    o = o_buf[...]
    for j in range(J_TAIL, N - 1):
        slot, e, st = j // 2 % SLOTS, j % 2, {}
        wait_filled(k_buf.at[slot, e], kv_sem(slot, e, 0))
        scores(st, j, nothing if j in QUIET else start_next)
        row_max(st)
        project_out(o, j - 1)
        wait_filled(v_buf.at[slot, e], kv_sem(slot, e, 1))
        attend(st, j, 0, HALF, start_next)
        o = normalized(st)
    assert not pending

    j = N - 1
    slot, e, st = j // 2 % SLOTS, j % 2, {}
    project_out(o, j - 1)
    wait_filled(k_buf.at[slot, e], kv_sem(slot, e, 0))
    scores(st, j, nothing)
    row_max(st)
    wait_filled(v_buf.at[slot, e, :, pl.ds(0, LAST_SPLIT)], kv_sem(slot, e, 1))
    for b in range(B - 1):
        pltpu.make_async_copy(out_buf.at[b], out_hbm.at[b], sems.at[SEM_OUT]).start(priority=b % 2)
    attend(st, j, 0, LAST_SPLIT, nothing)
    wait_filled(v_buf.at[slot, e, :, pl.ds(LAST_SPLIT, HALF - LAST_SPLIT)], sems.at[SEM_LAST])
    attend(st, j, LAST_SPLIT, HALF, nothing)
    project_out(normalized(st), j)
    pltpu.make_async_copy(out_buf.at[B - 1], out_hbm.at[B - 1], sems.at[SEM_OUT]).start()
    pltpu.make_async_copy(out_buf, out_hbm, sems.at[SEM_OUT]).wait()


@jax.jit
def pallas_standalone__mha_block_cached__near_ridge_kernel(
    x: jax.Array,
    k_cache: jax.Array,
    v_cache: jax.Array,
    wq: jax.Array,
    wo: jax.Array,
):
    assert x.shape == (B, SQ, D) and k_cache.shape == v_cache.shape == (B, H, SK, DH)
    dtype = x.dtype
    kv_shape = (2, 2, HALF, DH)
    w_shape = (W_GROUPS, D // W_GROUPS, H * DH)
    in_hbm = pl.BlockSpec(memory_space=pl.ANY)
    return pl.pallas_call(
        _kernel,
        in_specs=[in_hbm] * 5,
        out_specs=in_hbm,
        out_shape=jax.ShapeDtypeStruct((B, SQ, D), dtype),
        scratch_shapes=[
            pltpu.VMEM((SLOTS,) + kv_shape, dtype),
            pltpu.VMEM((SLOTS,) + kv_shape, dtype),
            pltpu.VMEM((B, SQ, D), dtype),
            pltpu.VMEM(w_shape, dtype),
            pltpu.VMEM(w_shape, dtype),
            pltpu.VMEM((N, SQ, DH), dtype),
            pltpu.VMEM((SQ, DH), dtype),
            pltpu.VMEM((SQ, D), jnp.float32),
            pltpu.VMEM((B, SQ, D), dtype),
            pltpu.SemaphoreType.DMA((NUM_SEMS,)),
        ],
        compiler_params=pltpu.CompilerParams(
            vmem_limit_bytes=100 * 1024 * 1024,
            disable_bounds_checks=True,
            disable_semaphore_checks=True,
        ),
    )(
        x,
        k_cache.reshape((N // 2,) + kv_shape),
        v_cache.reshape((N // 2,) + kv_shape),
        wq.reshape(w_shape),
        wo.T.reshape(w_shape),
    )
```

```python
import jax
import jax.numpy as jnp
from jax import lax
from jax.experimental import pallas as pl
from jax.experimental.pallas import tpu as pltpu

B, SQ, D = 8, 144, 448
H, SK, DH = 16, 2048, 256
N = B * H
HALF = SK // 2
PIECE = 32
BLOCK = 4 * PIECE
SLOTS = 8
KEYS = 256
W_GROUPS = 7
Q_SCALE = DH**-0.5 * 1.4426950408889634
NT = (((1,), (1,)), ((), ()))

J_PAIR = 114
J_HALF = 124
J_TAIL = 120
LEAD = 13
J_DROP = 105
SKEW = 26
QUIET = (121, 123, 125)
LAST_SPLIT = 640

SEM_W, SEM_LAST, SEM_OUT, NUM_SEMS = 4 * SLOTS, 4 * SLOTS + 3, 4 * SLOTS + 4, 4 * SLOTS + 5


def _window_positions(m, first, width, blocks):
    lanes, stagger = 4 // width, blocks // 4
    period = stagger * width
    positions = []
    for pos in range(4):
        w, sub = divmod(pos, lanes)
        turn = (m + stagger * (width - 1 - w)) >> (period.bit_length() - 1)
        positions.append((first + turn * width + w, (m & (period - 1)) * (BLOCK * lanes) + PIECE * sub, PIECE * lanes))
    return positions


def _run(obj, first_block, units):
    assert first_block % 4 == 0
    return [[(obj, BLOCK * ((first_block + 4 * u) % 16) + PIECE * pos, BLOCK) for pos in range(4)] for u in range(units)]


def _copies(kind, positions):
    return [(kind, kv, obj, row + step * t, kv) for t in range(4) for obj, row, step in positions for kv in (0, 1)]


def _make_plan():
    slabs = J_PAIR // 2
    left = 4 * (slabs - 3) % 16
    pair = [[(obj, BLOCK * (blk + m), PIECE) for obj, blk in ((0, 4), (0, 8), (1, 8), (2, 12))] for m in range(4)]
    pair += [[(obj, BLOCK * blk + PIECE * i, 2 * PIECE) for obj in (0, 1) for i in (0, 1)] for blk in (12, 14)]
    pair += [_window_positions(m, 0, 4, 16) for m in range(4 * (slabs - 3))]
    pair += _run(slabs - 3, left, 1) + _run(slabs - 2, left, 2) + _run(slabs - 1, left, 3)

    heads = J_HALF - J_PAIR
    half = _run(J_PAIR, 4, 1)
    half += [_window_positions(m, J_PAIR, 2, 8) for m in range(2 * (heads - 1))]
    half += _run(J_HALF - 1, 4 * (heads - 1) % 8, 1)

    rest = [("half", kv, j, row) for j in range(J_HALF, N) for kv in (0, 1) for row in range(0, HALF, PIECE)]
    queues = ([], [])
    for k, copy in enumerate(rest):
        if k >= len(rest) - 2 * SKEW:
            queue = int(k >= len(rest) - SKEW)
        else:
            queue = 0 if k < SKEW else (k - SKEW + 1) % 2
        queues[queue].append(copy + (queue,))
    rest = [q[k] for k in range(len(queues[0])) for q in queues if k < len(q)]

    units = [_copies("pair", p) for p in pair] + [_copies("half", p) for p in half]
    return pair, half, units + [rest[k : k + 32] for k in range(0, len(rest), 32)]


PAIR_UNITS, HALF_UNITS, UNITS = _make_plan()
J_SWITCH = (len(PAIR_UNITS) - LEAD + 1) // 2


def _half_units_before(j):
    return (3 * (j - J_SWITCH)) >> 1


def _check_plan():
    unit_of = {}
    for n, unit in enumerate(UNITS):
        for kind, kv, obj, row, _ in unit:
            for i in (0, 1):
                key = (kv, 2 * obj + i, row) if kind == "pair" else (kv, obj, i * HALF + row)
                assert key not in unit_of
                unit_of[key] = n
    assert set(unit_of) == {(kv, j, row) for kv in (0, 1) for j in range(N) for row in range(0, SK, PIECE)}
    assert LEAD + 2 * J_SWITCH - 1 == len(PAIR_UNITS) and _half_units_before(J_TAIL) < len(HALF_UNITS)
    assert 2 + 3 * (J_SWITCH // 2) >= N and J_DROP < J_SWITCH <= J_PAIR <= J_TAIL <= J_HALF
    started = LEAD
    for j in range(N):
        awaited = (j,) if j >= J_PAIR else (j & ~1, j | 1)
        assert all(unit_of[kv, i, row] < started for kv in (0, 1) for i in awaited for row in range(0, SK, PIECE))
        if j < J_SWITCH:
            count = 1 if j == J_DROP else 2
        elif j < J_TAIL:
            count = _half_units_before(j + 1) - _half_units_before(j)
        else:
            count = 0 if j == N - 1 else 1 if j in QUIET else 2
        for unit in UNITS[started : started + count]:
            assert all((obj if kind == "pair" else obj // 2) - SLOTS < j // 2 for kind, _, obj, _, _ in unit)
        started += count
    assert started >= len(UNITS)


_check_plan()


def _lane_fold(x, op):
    out = x[:, :128]
    for c in range(128, x.shape[1], 128):
        out = op(out, x[:, c : c + 128])
    return out


def _kernel(
    x_hbm, k_hbm, v_hbm, wq_hbm, wo_hbm, out_hbm,
    k_buf, v_buf, x_buf, wq_buf, wo_buf, q_buf, o_buf, acc, out_buf, sems,
):
    kv_hbm, kv_buf = (k_hbm, v_hbm), (k_buf, v_buf)

    def kv_sem(slot, e, kv):
        return sems.at[4 * slot + 2 * e + kv]

    def start_copy(kind, kv, obj, row, queue):
        if kind == "pair":
            slab, sem = obj, kv_sem(obj % SLOTS, 0, kv)
            ix = (slice(None), row // HALF, pl.ds(row % HALF, PIECE))
        else:
            slab, sem = obj // 2, kv_sem(obj // 2 % SLOTS, obj % 2, kv)
            ix = (obj % 2, slice(None), pl.ds(row, PIECE))
            if (kv, obj) == (1, N - 1) and row >= LAST_SPLIT:
                sem = sems.at[SEM_LAST]
        src, dst = kv_hbm[kv].at[(slab,) + ix], kv_buf[kv].at[(slab % SLOTS,) + ix]
        pltpu.make_async_copy(src, dst, sem).start(priority=queue)

    def start_unit(kind, m, positions, special, enabled=None):
        for k, other in special:
            positions = [tuple(jnp.where(m == k, a, b) for a, b in zip(p, q)) for p, q in zip(other, positions)]
        if kind == "pair":
            bases = [(obj, row >> 10, row & (HALF - 1), step) for obj, row, step in positions]
        else:
            bases = [(obj >> 1, obj & 1, row, step) for obj, row, step in positions]
        for t in range(4):
            for slab, mid, row, step in bases:
                rows, slot = pl.ds(pl.multiple_of(row + step * t, PIECE), PIECE), slab & (SLOTS - 1)
                ix = (slice(None), mid, rows) if kind == "pair" else (mid, slice(None), rows)

                def start():
                    for kv in (0, 1):
                        src, dst = kv_hbm[kv].at[(slab,) + ix], kv_buf[kv].at[(slot,) + ix]
                        sem = kv_sem(slot, 0 if kind == "pair" else mid, kv)
                        pltpu.make_async_copy(src, dst, sem).start(priority=kv)

                if enabled is None:
                    start()
                else:
                    pl.when(enabled)(start)

    def wait_filled(ref, sem):
        pltpu.make_async_copy(ref, ref, sem).wait()

    def head_cols(j):
        start = (j & (H - 1)) * DH
        return pl.ds(start if isinstance(start, int) else pl.multiple_of(start, DH), DH)

    def project_q(j):
        w = wq_buf[:, :, head_cols(j)].reshape(D, DH)
        q = jnp.dot(x_buf[j >> 4], w, preferred_element_type=jnp.float32)
        q_buf[j] = (q * Q_SCALE).astype(q_buf.dtype)

    def project_out(o, j):
        w = wo_buf[:, :, head_cols(j)].reshape(D, DH)
        y = lax.dot_general(o, w, NT, preferred_element_type=jnp.float32)
        if isinstance(j, int):
            y = y if j % H == 0 else acc[...] + y
            if j % H == H - 1:
                out_buf[j // H] = y.astype(out_buf.dtype)
            else:
                acc[...] = y
        else:
            y = jnp.where((j & (H - 1)) == 0, 0.0, acc[...]) + y
            acc[...] = y
            out_buf[j >> 4] = y.astype(out_buf.dtype)

    def key_chunks(lo, hi):
        return [(hf, r, min(KEYS, hi - r)) for hf in (0, 1) for r in range(lo, hi, KEYS)]

    def scores(st, j, midway):
        q = q_buf[j]
        for t, (hf, r, n) in enumerate(key_chunks(0, HALF)):
            k = k_buf[(j >> 1) & (SLOTS - 1), j & 1, hf, pl.ds(r, n), :]
            s = lax.dot_general(q, k, NT, preferred_element_type=jnp.float32)
            for c in range(0, n, 128):
                st[hf, r + c] = s[:, c : c + 128]
            top = _lane_fold(s, jnp.maximum)
            st["top"] = jnp.maximum(st["top"], top) if "top" in st else top
            if t == 3:
                midway()

    def row_max(st):
        if "max" not in st:
            st["max"] = jnp.max(st["top"], axis=-1, keepdims=True)
        return st["max"]

    def attend(st, j, lo, hi, midway):
        for t, (hf, r, n) in enumerate(key_chunks(lo, hi)):
            s = jnp.concatenate([st[hf, r + c] for c in range(0, n, 128)], axis=1)
            p = jnp.exp2(s - row_max(st))
            total = _lane_fold(p, jnp.add)
            st["sum"] = st["sum"] + total if "sum" in st else total
            v = v_buf[(j >> 1) & (SLOTS - 1), j & 1, hf, pl.ds(r, n), :]
            o = jnp.dot(p.astype(v.dtype), v, preferred_element_type=jnp.float32)
            st["o"] = st["o"] + o if "o" in st else o
            if t == 3:
                midway()

    def normalized(st):
        return (st["o"] * (1.0 / jnp.sum(st["sum"], axis=-1, keepdims=True))).astype(o_buf.dtype)

    def head(j, start_first, start_second):
        st = {}
        scores(st, j, start_first)
        project_out(o_buf[...], jnp.maximum(j - 1, 0))
        attend(st, j, 0, HALF, start_second)
        o_buf[...] = normalized(st)

    for r in range(0, D // W_GROUPS, 8):
        for c in range(0, H * DH, 1024):
            parts = [(pl.ds(g, 2), pl.ds(r, 8), pl.ds(c, 1024)) for g in range(0, W_GROUPS - 1, 2)]
            if c % 2048 == 0:
                parts.append((W_GROUPS - 1, pl.ds(r, 8), pl.ds(c, 2048)))
            for ix in parts:
                pltpu.make_async_copy(wq_hbm.at[ix], wq_buf.at[ix], sems.at[SEM_W]).start(priority=0)
                pltpu.make_async_copy(wo_hbm.at[ix], wo_buf.at[ix], sems.at[SEM_W + 1]).start(priority=1)
    x_parts = [(pl.ds(b, 2), pl.ds(r, 16)) for r in range(0, SQ, 16) for b in (0, 4, 2, 6)]
    for k, copy in enumerate(copy for unit in UNITS[:LEAD] for copy in unit):
        start_copy(*copy)
        if k % 8 == 7 and x_parts:
            for queue in (0, 1):
                ix = x_parts.pop(0)
                pltpu.make_async_copy(x_hbm.at[ix], x_buf.at[ix], sems.at[SEM_W + 2]).start(priority=queue)
    assert not x_parts
    acc[...] = jnp.zeros(acc.shape, acc.dtype)
    o_buf[...] = jnp.zeros(o_buf.shape, o_buf.dtype)
    for n, ref in enumerate((wq_buf, wo_buf, x_buf)):
        wait_filled(ref, sems.at[SEM_W + n])
    project_q(0)
    project_q(1)

    @pl.loop(0, J_SWITCH)
    def _(j):
        even, slot = (j & 1) == 0, (j >> 1) & (SLOTS - 1)
        ahead = 2 + 3 * (j >> 1)

        @pl.when(even & (ahead < N))
        def _():
            for t in range(3):
                project_q(ahead + t)

        @pl.when(even)
        def _():
            for kv in (0, 1):
                wait_filled(kv_buf[kv].at[slot], kv_sem(slot, 0, kv))

        def unit(m, enabled=None):
            drain = [(k, PAIR_UNITS[k]) for k in range(len(PAIR_UNITS) - 6, len(PAIR_UNITS))]
            start_unit("pair", m, _window_positions(m - 6, 0, 4, 16), drain, enabled)

        m = LEAD + 2 * j - jnp.where(j > J_DROP, 1, 0)
        head(j, lambda: unit(m), lambda: unit(m + 1, j != J_DROP))

    @pl.loop(J_SWITCH, J_TAIL)
    def _(j):
        slot, e = (j >> 1) & (SLOTS - 1), j & 1

        @pl.when((j < J_PAIR) & (e == 0))
        def _():
            for kv in (0, 1):
                wait_filled(kv_buf[kv].at[slot], kv_sem(slot, 0, kv))

        @pl.when(j >= J_PAIR)
        def _():
            for kv in (0, 1):
                wait_filled(kv_buf[kv].at[slot, e], kv_sem(slot, e, kv))

        def unit(m, enabled=None):
            start_unit("half", m, _window_positions(m - 1, J_PAIR, 2, 8), [(0, HALF_UNITS[0])], enabled)

        m = _half_units_before(j)
        head(j, lambda: unit(m), lambda: unit(m + 1, _half_units_before(j + 1) == m + 2))

    pending = UNITS[len(PAIR_UNITS) + _half_units_before(J_TAIL) :]

    def start_next():
        for copy in pending.pop(0) if pending else ():
            start_copy(*copy)

    def nothing():
        pass

    st = None
    for j in range(J_TAIL, N - 1):
        slot, e, previous, st = j // 2 % SLOTS, j % 2, st, {}
        wait_filled(k_buf.at[slot, e], kv_sem(slot, e, 0))
        scores(st, j, nothing if j in QUIET else start_next)
        row_max(st)
        project_out(normalized(previous) if previous else o_buf[...], j - 1)
        wait_filled(v_buf.at[slot, e], kv_sem(slot, e, 1))
        attend(st, j, 0, HALF, start_next)
    assert not pending

    j = N - 1
    project_out(normalized(st), j - 1)
    slot, e, st = j // 2 % SLOTS, j % 2, {}
    wait_filled(k_buf.at[slot, e], kv_sem(slot, e, 0))
    scores(st, j, nothing)
    row_max(st)
    wait_filled(v_buf.at[slot, e, :, pl.ds(0, LAST_SPLIT)], kv_sem(slot, e, 1))
    for b in range(B - 1):
        pltpu.make_async_copy(out_buf.at[b], out_hbm.at[b], sems.at[SEM_OUT]).start(priority=b % 2)
    attend(st, j, 0, LAST_SPLIT, nothing)
    wait_filled(v_buf.at[slot, e, :, pl.ds(LAST_SPLIT, HALF - LAST_SPLIT)], sems.at[SEM_LAST])
    attend(st, j, LAST_SPLIT, HALF, nothing)
    project_out(normalized(st), j)
    pltpu.make_async_copy(out_buf.at[B - 1], out_hbm.at[B - 1], sems.at[SEM_OUT]).start()
    pltpu.make_async_copy(out_buf, out_hbm, sems.at[SEM_OUT]).wait()


@jax.jit
def pallas_standalone__mha_block_cached__near_ridge_kernel(
    x: jax.Array,
    k_cache: jax.Array,
    v_cache: jax.Array,
    wq: jax.Array,
    wo: jax.Array,
):
    assert x.shape == (B, SQ, D) and k_cache.shape == v_cache.shape == (B, H, SK, DH)
    dtype = x.dtype
    kv_shape = (2, 2, HALF, DH)
    w_shape = (W_GROUPS, D // W_GROUPS, H * DH)
    in_hbm = pl.BlockSpec(memory_space=pl.ANY)
    return pl.pallas_call(
        _kernel,
        in_specs=[in_hbm] * 5,
        out_specs=in_hbm,
        out_shape=jax.ShapeDtypeStruct((B, SQ, D), dtype),
        scratch_shapes=[
            pltpu.VMEM((SLOTS,) + kv_shape, dtype),
            pltpu.VMEM((SLOTS,) + kv_shape, dtype),
            pltpu.VMEM((B, SQ, D), dtype),
            pltpu.VMEM(w_shape, dtype),
            pltpu.VMEM(w_shape, dtype),
            pltpu.VMEM((N, SQ, DH), dtype),
            pltpu.VMEM((SQ, DH), dtype),
            pltpu.VMEM((SQ, D), jnp.float32),
            pltpu.VMEM((B, SQ, D), dtype),
            pltpu.SemaphoreType.DMA((NUM_SEMS,)),
        ],
        compiler_params=pltpu.CompilerParams(
            vmem_limit_bytes=100 * 1024 * 1024,
            disable_bounds_checks=True,
            disable_semaphore_checks=True,
        ),
    )(
        x,
        k_cache.reshape((N // 2,) + kv_shape),
        v_cache.reshape((N // 2,) + kv_shape),
        wq.reshape(w_shape),
        wo.T.reshape(w_shape),
    )
```
